```python
import os as _os
_os.environ.setdefault("JAX_PLATFORMS", "cpu")
import jax
import jax.numpy as jnp

def _softmax(x, axis=-1):
    return jax.nn.softmax(x, axis=axis)
def _gelu(x):
    return jax.nn.gelu(x, approximate=True)
def _silu(x):
    return jax.nn.silu(x)
def _sigmoid(x):
    return jax.nn.sigmoid(x)
def _layernorm(x, axis=-1, eps=1e-5):
    m = jnp.mean(x, axis=axis, keepdims=True)
    v = jnp.var(x, axis=axis, keepdims=True)
    return (x - m) / jnp.sqrt(v + eps)
def _scatter_add(tgt, idx, src, axis=0):
    return tgt.at[idx].add(src)
def _segment_sum(src, seg, n):
    return jax.ops.segment_sum(src, seg, n)
class _Rng:
    def __init__(self, key):
        self._k = key
    def _next(self):
        self._k, sub = jax.random.split(self._k)
        return sub
    def normal(self, shape):
        return jax.random.normal(self._next(), shape, dtype=jnp.bfloat16)
    def randint(self, lo, hi, shape):
        return jax.random.randint(self._next(), shape, lo, hi, dtype=jnp.int32)
    def uniform(self, shape, lo=0.0, hi=1.0):
        return jax.random.uniform(self._next(), shape, jnp.bfloat16, lo, hi)
    def permutation(self, n):
        return jax.random.permutation(self._next(), n)


kernel_name = 'sequential_preLN__ssm_conv_h3__mixer_s_mlp__prompt'

def setup_inputs():
    _rng = _Rng(jax.random.key(int.from_bytes(__import__("os").urandom(4), "little")))
    _w = (lambda a: (lambda t: t.astype(jnp.bfloat16) if jnp.issubdtype(t.dtype, jnp.floating) else t)(jnp.asarray(a)))
    def _A_setup():
        B, S, D = 1, 2048, 640
        ks = 4
        return {
            "q": _w((lambda *s: _rng.normal(s) * 0.05)(B, S, D)),
            "k": _w((lambda *s: _rng.normal(s) * 0.05)(B, S, D)),
            "v": _w((lambda *s: _rng.normal(s) * 0.05)(B, S, D)),
            "shift_k": _w((lambda *s: _rng.normal(s) * 0.05)(D, ks) * 0.5),
            "ssm_k": _w((lambda *s: _rng.normal(s) * 0.05)(D, S) * (1.0 / S ** 0.5)),
            "ssm_D": _w((lambda *s: _rng.normal(s) * 0.05)(D)),
        }
    _A_in = _A_setup()

    def _B_setup():
        B, S, D, F = 1, 2048, 640, 1728
        return {
            "x":  _w((lambda *s: _rng.normal(s) * 0.05)(B, S, D)),
            "w1": _w((lambda *s: _rng.normal(s) * 0.8)(D, D) * (D ** -0.5)),
            "w2": _w((lambda *s: _rng.normal(s) * 0.8)(D, D) * (D ** -0.5)),
            "w3": _w((lambda *s: _rng.normal(s) * 0.8)(D, F) * (D ** -0.5)),
            "w4": _w((lambda *s: _rng.normal(s) * 0.8)(F, D) * (F ** -0.5)),
        }
    _B_in = _B_setup()

    return {
        "A_q": _A_in["q"],
        "A_k": _A_in["k"],
        "A_v": _A_in["v"],
        "A_shift_k": _A_in["shift_k"],
        "A_ssm_k": _A_in["ssm_k"],
        "A_ssm_D": _A_in["ssm_D"],
        "B_x": _B_in["x"],
        "B_w1": _B_in["w1"],
        "B_w2": _B_in["w2"],
        "B_w3": _B_in["w3"],
        "B_w4": _B_in["w4"],
    }

def reference(A_q, A_k, A_v, A_shift_k, A_ssm_k, A_ssm_D, B_x, B_w1, B_w2, B_w3, B_w4):
    def _A_ref(q, k, v, shift_k, ssm_k, ssm_D):
        B, S, D = q.shape
        ks = shift_k.shape[-1]
        k_pad = jnp.pad(k, ((0, 0), (ks - 1, 0), (0, 0)))
        k_shift = jnp.zeros_like(k)
        for t in range(ks):
            k_shift = k_shift + k_pad[:, t:t + S, :] * shift_k[:, ks - 1 - t][None, None, :]
        kv = k_shift * v
        L = 2 * S
        kv_pad = jnp.pad(kv, ((0, 0), (0, S), (0, 0)))
        kf_pad = jnp.pad(ssm_k, ((0, 0), (0, S)))
        kv_f = (lambda x, axes=(-2,-1): jnp.fft.rfft2(x.astype(jnp.float32), axes=axes))(kv_pad[:, None, :, :], axes=(1, 2))
        kf_f = (lambda x, axes=(-2,-1): jnp.fft.rfft2(x.astype(jnp.float32), axes=axes))(kf_pad[:, None, :], axes=(1, 2))
        kf_f = (lambda x, *d: x.transpose(*d))(kf_f, 1, 2, 0)
        y_f = kv_f * kf_f[None, :, :, :]
        y = (lambda x, s, axes=(-2,-1): jnp.fft.irfft2(x, s=s, axes=axes).astype(jnp.bfloat16))(y_f, (1, L), axes=(1, 2))[:, 0, :S, :]
        y = y + kv * ssm_D[None, None, :]
        return q * y

    def _B_ref(x, w1, w2, w3, w4):
        B, S, D = x.shape
        h = _gelu(_layernorm(x, axis=-1) @ w1)
        c = D // 4
        g0 = jnp.pad(h[:, :, 0*c:1*c], ((0, 0), (1, 0), (0, 0)))[:, :S, :]
        g1 = jnp.pad(h[:, :, 1*c:2*c], ((0, 0), (0, 1), (0, 0)))[:, 1:, :]
        g2 = jnp.pad(h[:, :, 2*c:3*c], ((0, 0), (2, 0), (0, 0)))[:, :S, :]
        g3 = jnp.pad(h[:, :, 3*c:   ], ((0, 0), (0, 2), (0, 0)))[:, 2:, :]
        hs = jnp.concatenate([g0, g1, g2, g3], axis=-1) @ w2
        x1 = x + hs
        h2 = _gelu(_layernorm(x1, axis=-1) @ w3) @ w4
        return x1 + h2

    x = A_q
    h = x + _A_ref(_layernorm(x, axis=-1), A_k, A_v, A_shift_k, A_ssm_k, A_ssm_D)
    h2 = h + _B_ref(_layernorm(h, axis=-1), B_w1, B_w2, B_w3, B_w4)
    return h2
```

```python
import functools
import os
import numpy as np
import ml_dtypes
import jax
import jax.numpy as jnp
import jax.experimental.pallas as pl
import jax.experimental.pallas.tpu as pltpu

S, D, F = 2048, 640, 1728
TM = 256
NT = S // TM
SK = 16
ACH = 32
LAG = 3
f32, bf16, u32 = jnp.float32, jnp.bfloat16, jnp.uint32


i32 = jnp.int32


def _cmul(a, b):
    return a[0]*b[0] - a[1]*b[1], a[0]*b[1] + a[1]*b[0]


def _cis(m):
    mm = (m & 8191) + 1024
    q = mm >> 11
    x = ((mm & 2047) - 1024).astype(f32) * np.float32(2*np.pi/8192)
    x2 = x*x
    s = x + x*x2*(np.float32(-1/6) + x2*(np.float32(1/120) + x2*(np.float32(-1/5040) + x2*np.float32(1/362880))))
    c = 1.0 + x2*(np.float32(-1/2) + x2*(np.float32(1/24) + x2*(np.float32(-1/720) + x2*(np.float32(1/40320) + x2*np.float32(-1/3628800)))))
    odd = (q & 1) == 1
    cs = jnp.where(odd, s, c); sn = jnp.where(odd, c, s)
    cs = jnp.where(((q + 1) & 2) != 0, -cs, cs)
    sn = jnp.where((q & 2) != 0, -sn, sn)
    return cs, sn


def _dot(a, b):
    return jnp.dot(a, b, preferred_element_type=f32)

def _dot_t(a, b):
    return jax.lax.dot_general(a, b, (((1,), (1,)), ((), ())), preferred_element_type=f32)

def _tob(w):
    return pltpu.bitcast(w, bf16)

def _pk(a, b):
    return pltpu.pack_elementwise([a, b], packed_dtype=bf16)

def _mo(v, m):
    return v if isinstance(v, int) else pl.multiple_of(v, m)

def _ln(x):
    m = jnp.sum(x, axis=-1, keepdims=True) * (1.0/D)
    c = x - m
    v = jnp.sum(c*c, axis=-1, keepdims=True) * (1.0/D)
    return c * jax.lax.rsqrt(v + 1e-5)

def _gelu(x):
    return (0.5*x)*(1.0 + jnp.tanh(x*(0.7978845608028654 + (0.7978845608028654*0.044715)*(x*x))))


def _kernel(q_hbm, k_hbm, v_hbm, sk_hbm, h_hbm, d_hbm, w1_hbm, w2_hbm, w3_hbm, w4_hbm,
            o_hbm,
            k_s, v_s, hf_s, sk_s, d_s, skf_s, G_s, H_s, HI_s, GI_s, kv_s, ht_s, s2_s, s3_s, z_s, y_s,
            q_s, w1_s, w2_s, w3_s, w4_s, h_s, xp_s, a_s, hh_s, res_s, o_s,
            sem, sem_o):
    def cp_k(c): return pltpu.make_async_copy(k_hbm.at[:, pl.ds(_mo(c*128, 128), 128)], k_s.at[c], sem.at[c])
    def cp_v(c): return pltpu.make_async_copy(v_hbm.at[:, pl.ds(_mo(c*128, 128), 128)], v_s.at[c], sem.at[5+c])
    def cp_h(c): return pltpu.make_async_copy(h_hbm.at[pl.ds(_mo(c*128, 128), 128), :], hf_s.at[c], sem.at[10+c])
    cp_sk = pltpu.make_async_copy(sk_hbm, sk_s, sem.at[15])
    cp_d = pltpu.make_async_copy(d_hbm, d_s, sem.at[16])
    NQ = 4
    QR = S // NQ
    cp_q = [pltpu.make_async_copy(q_hbm.at[pl.ds(i*QR, QR), :], q_s.at[pl.ds(i*QR, QR), :], sem.at[21+i]) for i in range(NQ)]
    cp_w = []
    for wi, (w_hbm, w_s) in enumerate(((w1_hbm, w1_s), (w2_hbm, w2_s), (w3_hbm, w3_s), (w4_hbm, w4_s))):
        wv = w_s.bitcast(bf16)
        cp_w.append([pltpu.make_async_copy(w_hbm.at[:, pl.ds(128*n, 128)], wv.at[n], sem.at[25+5*wi+n]) for n in range(5)])

    for cp in (cp_h(0), cp_k(0), cp_v(0), cp_sk, cp_d, cp_k(1), cp_v(1), cp_h(1)):
      cp.start()
    for c in range(2, 5):
      cp_k(c).start(); cp_v(c).start(); cp_h(c).start()
    cp_q[0].start()
    for wi in range(4):
      for cp in cp_w[wi]:
          cp.start()
    for i in range(1, NQ):
      cp_q[i].start()


    def gen_G():
        lane = jax.lax.broadcasted_iota(i32, (128, 128), 1)
        row = jax.lax.broadcasted_iota(i32, (128, 128), 0)
        k1 = row >> 3; ri = (row >> 2) & 1; rr = row & 3
        j = 2*(lane >> 4) + (lane & 1); rp = (lane >> 1) & 7
        for lh in range(2):
            m = (4*k1 + 1)*(2*j + lh)*64 - 2048*ri
            v = _cis(m)[0]
            G_s[lh] = _pk(jnp.where(2*rr == rp, v, 0.0), jnp.where(2*rr + 1 == rp, v, 0.0))
    def gen_GI():
        lane = jax.lax.broadcasted_iota(i32, (64, 256), 1)
        row = jax.lax.broadcasted_iota(i32, (64, 256), 0)
        j = row >> 2; rr = row & 3
        k1 = lane >> 4; r = (lane >> 1) & 7; ri = lane & 1
        for lh in range(2):
            m = (4*k1 + 1)*(2*j + lh)*64 - 2048*ri
            v = _cis(m)[0] * (1.0/S)
            GI_s[lh] = _pk(jnp.where(2*rr == r, v, 0.0), jnp.where(2*rr + 1 == r, v, 0.0))
    def gen_H():
        lane = jax.lax.broadcasted_iota(i32, (32, 128), 1)
        row = jax.lax.broadcasted_iota(i32, (32, 128), 0)
        l = lane >> 1; ri = lane & 1
        u = _cis(4*l[0:8]); u = tuple(jnp.concatenate([x]*4, axis=0) for x in u)
        W = [_cis((1 + 256*row + 128*p)*l + 2048*ri) for p in range(2)]
        for n in range(32):
            idx = 2*(n % 16) + n // 16
            H_s[idx, 0:32, :] = _pk(W[0][0], W[1][0])
            H_s[idx, 32:64, :] = _pk(W[0][1], W[1][1])
            if n < 31: W = [_cmul(w, u) for w in W]
        k2 = lane & 63; rip = lane >> 6
        T = [_cis(-4*(2*row + p)) for p in range(2)]
        W = [_cis(-(1 + 128*k2)*(2*row + p) + 2048*rip) for p in range(2)]
        for n in range(32):
            idx = 2*(n % 16) + n // 16
            HI_s[idx, 0:32, :] = _pk(W[0][0], W[1][0])
            HI_s[idx, 32:64, :] = _pk(W[0][1], W[1][1])
            if n < 31: W = [_cmul(w, t) for w, t in zip(W, T)]
    gen_G(); gen_H(); gen_GI()

    z_s[...] = jnp.zeros((8, 128), u32)
    hh_s[:, 0:8, :] = jnp.zeros((5, 8, 128), f32)
    q_s[S:S+SK, :] = jnp.zeros((SK, D), bf16)
    y_s[S:S+SK, :] = jnp.zeros((SK, D), f32)

    def P(c):
        cs = pl.ds(_mo(c*128, 128), 128)
        w = [skf_s[i:i+1, cs] for i in range(4)]
        kfs = [k_s[c, 128*j:128*(j+1), :].astype(f32) for j in range(16)]
        def kvt(j):
            prev = kfs[j-1][120:128] if j else jnp.zeros((8, 128), f32)
            win = jnp.concatenate([prev, kfs[j]], axis=0)
            ks = w[3]*win[5:133] + w[2]*win[6:134] + w[1]*win[7:135] + w[0]*kfs[j]
            return ks * v_s[c, 128*j:128*(j+1), :].astype(f32)
        ties = []
        for jp in range(8):
            p = _pk(kvt(2*jp), kvt(2*jp+1)).reshape(16, 8, 128)
            kv_s[:, jp] = p
            ties += [pltpu.bitcast(p[i] & z_s[...], f32) for i in range(16)]
            ha = hf_s[c, :, 256*jp:256*jp+128].astype(f32)
            hb = hf_s[c, :, 256*jp+128:256*jp+256].astype(f32)
            ht_s[:, jp] = _pk(ha, hb).T.reshape(16, 8, 128)
        return ties

    def S1():
        for src, buf in enumerate((kv_s, ht_s)):
            for g in range(8):
                lo = _dot(_tob(G_s[0]), _tob(buf[g].reshape(64, 128)))
                hi = _dot(_tob(G_s[1]), _tob(buf[8+g].reshape(64, 128)))
                for par, e in enumerate((lo+hi, lo-hi)):
                    e = e.reshape(16, 2, 8, 128)
                    s2_s[src, par, :, g] = _pk(e[:, 0], e[:, 1])

    def S2(c, ties):
        cs = pl.ds(_mo(c*128, 128), 128)
        dd = skf_s[4:5, cs]
        TIE0 = 2
        NP = 32 - TIE0
        def AB(k1):
            Ys = []
            for par in range(2):
                Hm = _tob(H_s[2*k1+par])
                A = _dot(Hm, _tob(s2_s[0, par, k1].reshape(64, 128)))
                B = _dot(Hm, _tob(s2_s[1, par, k1].reshape(64, 128)))
                Ar, Ai, Br, Bi = A[:64], A[64:], B[:64] + dd, B[64:]
                Yr = Ar*Br - Ai*Bi
                Yi = Ar*Bi + Ai*Br
                if ties:
                    n = 2*k1 + par
                    mine = [t for qi, t in enumerate(ties) if (qi*NP)//len(ties) + TIE0 == n]
                    rows = [Yr[8*i:8*i+8] for i in range(8)]
                    for i, t in enumerate(mine):
                        rows[i % 8] = rows[i % 8] + t
                    Yr = jnp.concatenate(rows, axis=0)
                Ys.append(jnp.concatenate([Yr, Yi], axis=0).astype(bf16))
            return Ys
        def DD(k1, Ys):
            Dd = [_dot(_tob(HI_s[2*k1+par]), Ys[par]) for par in range(2)]
            for lh, e in enumerate((Dd[0] + Dd[1], Dd[0] - Dd[1])):
                s3_s[lh, :, k1] = _pk(e[0:64], e[64:128]).reshape(8, 8, 128)
        pend = {}
        for k1 in range(16 + LAG):
            if k1 < 16:
                pend[k1] = AB(k1)
            if k1 - LAG >= 0:
                DD(k1 - LAG, pend.pop(k1 - LAG))

    def S3(c):
        cs = pl.ds(_mo(c*128, 128), 128)
        for lh in range(2):
            for g in range(8):
                o = _dot(_tob(GI_s[lh]), _tob(s3_s[lh, g].reshape(128, 128)))
                l0 = 64*lh + 8*g
                for j in range(16):
                    y_s[128*j+l0:128*j+l0+8, cs] = o[8*j:8*j+8]

    cp_h(0).wait(); cp_k(0).wait(); cp_v(0).wait()
    cp_sk.wait(); cp_d.wait()
    skf_s[0:4, :] = sk_s[...].astype(f32)
    skf_s[4:5, :] = d_s[...].astype(f32).reshape(1, D)
    P(0); S1()
    def conv_body(c, carry):
        cp_k(c+1).wait(); cp_v(c+1).wait(); cp_h(c+1).wait()
        ties = P(c+1); S2(c, ties); S1(); S3(c)
        return carry
    jax.lax.fori_loop(0, 4, conv_body, 0)
    S2(4, None); S3(4)

    lane = jax.lax.broadcasted_iota(jnp.int32, (TM, 128), 1)

    def A(r0, nrows):
        for j in range(0, nrows, ACH):
            n = min(ACH, nrows - j)
            r = pl.ds(_mo(r0 + j, 16), n)
            x = q_s[r, :].astype(f32)
            h = x + _ln(x)*y_s[r, :]
            h_s[r, :] = h
            xp = _ln(h)
            xp_s[r, :] = xp
            a_s[r, :] = _ln(xp)

    def M1(r0, nrows):
        r = pl.ds(r0, nrows)
        av = [a_s[r, k*128:(k+1)*128].astype(bf16) for k in range(5)]
        for n in range(5):
            acc = None
            for k in range(5):
                p = _dot(av[k], _tob(w1_s[n, k*64:(k+1)*64, :]))
                acc = p if acc is None else acc + p
            hh_s[n, pl.ds(r0+8, nrows), :] = _gelu(acc)

    def M2(base):
        r = pl.ds(base, TM)
        def sh(n, s): return hh_s.at[n, pl.ds(base, TM+16), :][8-s:8-s+TM, :]
        gs = [sh(0, 1),
              jnp.where(lane < 32, sh(1, 1), sh(1, -1)),
              jnp.where(lane < 64, sh(2, -1), sh(2, 2)),
              jnp.where(lane < 96, sh(3, 2), sh(3, -2)),
              sh(4, -2)]
        gs = [g.astype(bf16) for g in gs]
        x1s = []
        for n in range(5):
            acc = None
            for k in range(5):
                p = _dot(gs[k], _tob(w2_s[n, k*64:(k+1)*64, :]))
                acc = p if acc is None else acc + p
            x1s.append(xp_s[r, n*128:(n+1)*128] + acc)
        x1 = jnp.concatenate(x1s, axis=1)
        res_s[...] = h_s[r, :] + x1
        return _ln(x1)

    def M3(b):
        bs = [b[:, k*128:(k+1)*128].astype(bf16) for k in range(5)]
        gs = []
        for n in range(14):
            lo, hi = n*64, min((n+1)*64, F//2)
            acc = None
            for k in range(5):
                p = _dot_t(bs[k], _tob(w3_s[k, lo:hi, :]))
                acc = p if acc is None else acc + p
            gs.append(_gelu(acc).astype(bf16))
        return gs

    def M4(slot, gs):
        for n in range(5):
            acc = None
            for k in range(14):
                lo, hi = k*64, min((k+1)*64, F//2)
                p = _dot(gs[k], _tob(w4_s[n, lo:hi, :]))
                acc = p if acc is None else acc + p
            cs = slice(n*128, (n+1)*128)
            o_s[slot, :, cs] = (res_s[:, cs] + acc).astype(bf16)

    def cp_o(i, slot):
        return pltpu.make_async_copy(o_s.at[slot], o_hbm.at[pl.ds(_mo(i*TM, TM), TM), :], sem_o.at[slot])

    cp_q[0].wait()
    for cp in cp_w[0]: cp.wait()
    cp_q[1].wait()
    A(0, TM+SK); M1(0, TM+SK)
    A(TM+SK, TM)
    for wi in (1, 2, 3):
        for cp in cp_w[wi]: cp.wait()
    for i in range(2, NQ):
        cp_q[i].wait()

    def mlp_body(i, carry):
        slot = i % 2
        @pl.when(i >= 2)
        def _():
            cp_o(i-2, slot).wait()
        base = _mo(i*TM, TM)
        a1 = _mo((i+1)*TM+SK, SK)
        a2 = _mo(jnp.minimum(i+2, NT-1)*TM+SK, SK)
        b = M2(base); M1(a1, TM); gs = M3(b); A(a2, TM); M4(slot, gs)
        cp_o(i, slot).start()
        return carry
    jax.lax.fori_loop(0, NT-1, mlp_body, 0)
    i = NT-1
    cp_o(i-2, i % 2).wait()
    b = M2(i*TM)
    M4(i % 2, M3(b))
    cp_o(i, i % 2).start()
    cp_o(i-1, (i-1) % 2).wait()
    cp_o(i, i % 2).wait()


def _hbm(x):
    return pltpu.with_memory_space_constraint(x, pltpu.HBM)


@jax.jit
def pallas_sequential_preLN__ssm_conv_h3__mixer_s_mlp__prompt_kernel(
    A_q, A_k, A_v, A_shift_k, A_ssm_k, A_ssm_D, B_x, B_w1, B_w2, B_w3, B_w4):
    del B_x
    args = (A_q.reshape(S, D), A_k.reshape(S, D), A_v.reshape(S, D), A_shift_k.T, A_ssm_k, A_ssm_D,
            B_w1, B_w2, B_w3.T, B_w4)
    out = pl.pallas_call(
        _kernel,
        out_shape=jax.ShapeDtypeStruct((S, D), bf16),
        in_specs=[pl.BlockSpec(memory_space=pltpu.HBM)] * len(args),
        out_specs=pl.BlockSpec(memory_space=pltpu.HBM),
        scratch_shapes=[
            pltpu.VMEM((5, S, 128), bf16), pltpu.VMEM((5, S, 128), bf16), pltpu.VMEM((5, 128, S), bf16),
            pltpu.VMEM((4, D), bf16), pltpu.VMEM((D,), bf16), pltpu.VMEM((8, D), f32),
            pltpu.VMEM((2, 128, 128), u32), pltpu.VMEM((32, 64, 128), u32), pltpu.VMEM((32, 64, 128), u32), pltpu.VMEM((2, 64, 256), u32),
            pltpu.VMEM((16, 8, 8, 128), u32), pltpu.VMEM((16, 8, 8, 128), u32),
            pltpu.VMEM((2, 2, 16, 8, 8, 128), u32), pltpu.VMEM((2, 8, 16, 8, 128), u32),
            pltpu.VMEM((8, 128), u32), pltpu.VMEM((S+SK, D), f32),
            pltpu.VMEM((S+SK, D), bf16),
            pltpu.VMEM((5, D//2, 128), u32), pltpu.VMEM((5, D//2, 128), u32), pltpu.VMEM((5, F//2, 128), u32), pltpu.VMEM((5, F//2, 128), u32),
            pltpu.VMEM((S+SK, D), f32), pltpu.VMEM((S+SK, D), f32), pltpu.VMEM((S+SK, D), f32),
            pltpu.VMEM((5, S+SK+16, 128), f32), pltpu.VMEM((TM, D), f32), pltpu.VMEM((2, TM, D), bf16),
            pltpu.SemaphoreType.DMA((45,)), pltpu.SemaphoreType.DMA((2,)),
        ],
        compiler_params=pltpu.CompilerParams(vmem_limit_bytes=100*2**20),
        name="ssm_mixer_block",
    )(*[_hbm(a) for a in args])
    return out.reshape(1, S, D)
```

```python
import contextlib
import numpy as np
import jax
import jax.numpy as jnp
import jax.experimental.pallas as pl
import jax.experimental.pallas.tpu as pltpu

S, D, F = 2048, 640, 1728
TM = 256
NT = S // TM
SK = 16
ACH = 32
_DEF = dict(SLAB='1', PRE='1', T0='4', T1='60', FV='1', BAR='1', CH='0', F0='12', F1='48', DF='1', TIE0='1', HW2='1')
E = lambda k, d=None: _DEF.get(k, d)
LAG = int(E("LAG", "3"))
TIE0 = int(E("TIE0", "2"))
T0 = int(E("T0", "6")); T1 = int(E("T1", "62"))
f32, bf16, u32, i32 = jnp.float32, jnp.bfloat16, jnp.uint32, jnp.int32
scope = (lambda n: jax.named_scope(n)) if E("SCOPES") else (lambda n: contextlib.nullcontext())


def _cmul(a, b):
    return a[0]*b[0] - a[1]*b[1], a[0]*b[1] + a[1]*b[0]


def _cis(m):
    mm = (m & 8191) + 1024
    q = mm >> 11
    x = ((mm & 2047) - 1024).astype(f32) * np.float32(2*np.pi/8192)
    x2 = x*x
    s = x + x*x2*(np.float32(-1/6) + x2*(np.float32(1/120) + x2*(np.float32(-1/5040) + x2*np.float32(1/362880))))
    c = 1.0 + x2*(np.float32(-1/2) + x2*(np.float32(1/24) + x2*(np.float32(-1/720) + x2*(np.float32(1/40320) + x2*np.float32(-1/3628800)))))
    odd = (q & 1) == 1
    cs = jnp.where(odd, s, c); sn = jnp.where(odd, c, s)
    cs = jnp.where(((q + 1) & 2) != 0, -cs, cs)
    sn = jnp.where((q & 2) != 0, -sn, sn)
    return cs, sn


def sadd(a, b):
    (sa, xa), (sb, xb) = a, b
    if sa == sb: return (sa, xa + xb)
    return (1, xa - xb) if sa > 0 else (1, xb - xa)
def sneg(a): return (-a[0], a[1])
def ssub(a, b): return sadd(a, sneg(b))
def smul(a, c):
    c = float(c)
    return (a[0]*(1 if c > 0 else -1), a[1]*np.float32(abs(c)))
def val(a):
    if a[0] > 0: return a[1]
    return -a[1]
def cadd(a, b): return (sadd(a[0], b[0]), sadd(a[1], b[1]))
def csub(a, b): return (ssub(a[0], b[0]), ssub(a[1], b[1]))
def cmuli(a): return (sneg(a[1]), a[0])
def bfly4(z0, z1, z2, z3):
    t0, t1, t2, t3 = cadd(z0, z2), csub(z0, z2), cadd(z1, z3), csub(z1, z3)
    it3 = cmuli(t3)
    return cadd(t0, t2), cadd(t1, it3), csub(t0, t2), csub(t1, it3)
def ctw(a, k):
    k %= 16
    if k == 0: return a
    if k == 4: return cmuli(a)
    if k == 8: return (sneg(a[0]), sneg(a[1]))
    if k == 12: return (a[1], sneg(a[0]))
    c, s = np.cos(2*np.pi*k/16), np.sin(2*np.pi*k/16)
    if k % 2 == 0:
        r = sadd((a[0][0]*int(np.sign(c)), a[0][1]), (-a[1][0]*int(np.sign(s)), a[1][1]))
        i = sadd((a[0][0]*int(np.sign(s)), a[0][1]), (a[1][0]*int(np.sign(c)), a[1][1]))
        return (smul(r, abs(c)), smul(i, abs(c)))
    return (ssub(smul(a[0], c), smul(a[1], s)), sadd(smul(a[0], s), smul(a[1], c)))
def fft16(z):
    u = [bfly4(z[n1], z[4+n1], z[8+n1], z[12+n1]) for n1 in range(4)]
    X = [None]*16
    for m1 in range(4):
        v = [ctw(u[n1][m1], m1*n1) for n1 in range(4)]
        o = bfly4(*v)
        for m2 in range(4): X[m1 + 4*m2] = o[m2]
    return X
def branch(a, b):
    e1, e2 = (1, 16) if b == 0 else (5, 80)
    z = []
    for n in range(16):
        a0, a1 = (1, a[n]), (1, a[n+16])
        if n == 0:
            c = np.cos(2*np.pi*e2/128); s = np.sin(2*np.pi*e2/128)
            t = smul(a1, abs(c))
            z.append((sadd(a0, (t[0]*int(np.sign(c)), t[1])), (t[0]*int(np.sign(s)), t[1])))
        else:
            al, be = 2*np.pi*(e1*n)/128, 2*np.pi*(e1*n + e2)/128
            z.append((sadd(smul(a0, np.cos(al)), smul(a1, np.cos(be))), sadd(smul(a0, np.sin(al)), smul(a1, np.sin(be)))))
    X = fft16(z)
    return [(val(x[0]), val(x[1])) for x in X]


def _dot(a, b):
    return jnp.dot(a, b, preferred_element_type=f32)

def _dot_t(a, b):
    return jax.lax.dot_general(a, b, (((1,), (1,)), ((), ())), preferred_element_type=f32)

def _tob(w):
    return pltpu.bitcast(w, bf16)

def _pk(a, b):
    return pltpu.pack_elementwise([a, b], packed_dtype=bf16)

def _mo(v, m):
    return v if isinstance(v, int) else pl.multiple_of(v, m)

def _ln(x):
    m = jnp.sum(x, axis=-1, keepdims=True) * (1.0/D)
    c = x - m
    v = jnp.sum(c*c, axis=-1, keepdims=True) * (1.0/D)
    return c * jax.lax.rsqrt(v + 1e-5)

def _gelu(x):
    return (0.5*x)*(1.0 + jnp.tanh(x*(0.7978845608028654 + (0.7978845608028654*0.044715)*(x*x))))


def _kernel(q_hbm, k_hbm, v_hbm, sk_hbm, h_hbm, d_hbm, w1_hbm, w2_hbm, w3_hbm, w4_hbm, o_hbm,
            k_s, v_s, hf_s, sk_s, d_s, skf_s, G_s, H_s, HI_s, GI_s, kv_s, ht_s, s2_s, s3_s, z_s, y_s,
            kf_s, hT_s, q_s, w1_s, w2_s, w3_s, w4_s, h_s, xp_s, a_s, hh_s, res_s, o_s,
            flag_s, sem, sem_o):
    def cp_k(c): return pltpu.make_async_copy(k_hbm.at[:, pl.ds(_mo(c*128, 128), 128)], k_s.at[c], sem.at[c])
    def cp_v(c): return pltpu.make_async_copy(v_hbm.at[:, pl.ds(_mo(c*128, 128), 128)], v_s.at[c], sem.at[5+c])
    def cp_h(c): return pltpu.make_async_copy(h_hbm.at[pl.ds(_mo(c*128, 128), 128), :], hf_s.at[c], sem.at[10+c])
    cp_sk = pltpu.make_async_copy(sk_hbm, sk_s, sem.at[15])
    cp_d = pltpu.make_async_copy(d_hbm, d_s, sem.at[16])
    QB = (0, 640, S)
    cp_q = [pltpu.make_async_copy(q_hbm.at[pl.ds(QB[i], QB[i+1]-QB[i]), :], q_s.at[pl.ds(QB[i], QB[i+1]-QB[i]), :], sem.at[17+i])
            for i in range(2)]
    cp_w = []
    for wi, (w_hbm, w_s) in enumerate(((w1_hbm, w1_s), (w2_hbm, w2_s), (w3_hbm, w3_s), (w4_hbm, w4_s))):
        wv = w_s.bitcast(bf16)
        cp_w.append([pltpu.make_async_copy(w_hbm.at[:, pl.ds(128*n, 128)], wv.at[n], sem.at[19+5*wi+n]) for n in range(5)])
    def cp_o(i, slot):
        return pltpu.make_async_copy(o_s.at[slot], o_hbm.at[pl.ds(_mo(i*TM, TM), TM), :], sem_o.at[slot])
    def cp_slab(i, n):
        return pltpu.make_async_copy(o_s.at[i % 2, :, pl.ds(128*n, 128)], o_hbm.at[pl.ds(i*TM, TM), pl.ds(128*n, 128)], sem_o.at[2+n])

    with scope("s0_issue"):
        for cp in (cp_h(0), cp_sk, cp_d, cp_k(0), cp_v(0), cp_k(1), cp_v(1), cp_h(1)):
            cp.start()
        for c in range(2, 5):
            cp_k(c).start(); cp_v(c).start(); cp_h(c).start()
        cp_q[0].start()
        for wi in range(4):
            for cp in cp_w[wi]:
                cp.start()
        cp_q[1].start()

    def gen_G():
        lane = jax.lax.broadcasted_iota(i32, (128, 128), 1)
        row = jax.lax.broadcasted_iota(i32, (128, 128), 0)
        k1 = row >> 3; ri = (row >> 2) & 1; rr = row & 3
        j = 2*(lane >> 4) + (lane & 1); rp = (lane >> 1) & 7
        for lh in range(2):
            v = _cis((4*k1 + 1)*(2*j + lh)*64 - 2048*ri)[0]
            G_s[lh] = _pk(jnp.where(2*rr == rp, v, 0.0), jnp.where(2*rr + 1 == rp, v, 0.0))
    def gen_GI():
        lane = jax.lax.broadcasted_iota(i32, (64, 256), 1)
        row = jax.lax.broadcasted_iota(i32, (64, 256), 0)
        j = row >> 2; rr = row & 3
        k1 = lane >> 4; r = (lane >> 1) & 7; ri = lane & 1
        for lh in range(2):
            v = _cis((4*k1 + 1)*(2*j + lh)*64 - 2048*ri)[0] * (1.0/S)
            GI_s[lh] = _pk(jnp.where(2*rr == r, v, 0.0), jnp.where(2*rr + 1 == r, v, 0.0))
    def gen_H():
        lane = jax.lax.broadcasted_iota(i32, (32, 128), 1)
        row = jax.lax.broadcasted_iota(i32, (32, 128), 0)
        l = lane >> 1; ri = lane & 1
        u = _cis(4*l[0:8]); u = tuple(jnp.concatenate([x]*4, axis=0) for x in u)
        W = [_cis((1 + 256*row + 128*p)*l + 2048*ri) for p in range(2)]
        for n in range(32):
            idx = 2*(n % 16) + n // 16
            H_s[idx, 0:32, :] = _pk(W[0][0], W[1][0])
            H_s[idx, 32:64, :] = _pk(W[0][1], W[1][1])
            if n < 31: W = [_cmul(w, u) for w in W]
        k2 = lane & 63; rip = lane >> 6
        T = [_cis(-4*(2*row + p)) for p in range(2)]
        W = [_cis(-(1 + 128*k2)*(2*row + p) + 2048*rip) for p in range(2)]
        for n in range(32):
            idx = 2*(n % 16) + n // 16
            HI_s[idx, 0:32, :] = _pk(W[0][0], W[1][0])
            HI_s[idx, 32:64, :] = _pk(W[0][1], W[1][1])
            if n < 31: W = [_cmul(w, t) for w, t in zip(W, T)]
    with scope("s0b_gen"):
        gen_G(); gen_H(); gen_GI()
        flag_s[0] = 1
        kf_s[0:8, :] = jnp.zeros((8, 128), f32)
        z_s[...] = jnp.zeros((8, 128), u32)
        hh_s[:, 0:8, :] = jnp.zeros((5, 8, 128), f32)
        q_s[S:S+SK, :] = jnp.zeros((SK, D), bf16)
        y_s[S:S+SK, :] = jnp.zeros((SK, D), f32)

    def P(c):
        cs = pl.ds(_mo(c*128, 128), 128)
        w = [skf_s[i:i+1, cs] for i in range(4)]
        kfs = [k_s[c, 128*j:128*(j+1), :].astype(f32) for j in range(16)]
        if E("UL"):
            for j in range(16):
                kf_s[8+128*j:8+128*(j+1), :] = kfs[j]
        def kvt(j):
            prev = kfs[j-1][120:128] if j else jnp.zeros((8, 128), f32)
            win = jnp.concatenate([prev, kfs[j]], axis=0)
            if E("UL"):
                b = 8 + 128*j
                ks = w[3]*kf_s[b-3:b+125, :] + w[2]*kf_s[b-2:b+126, :] + w[1]*kf_s[b-1:b+127, :] + w[0]*kfs[j]
            else:
                ks = w[3]*win[5:133] + w[2]*win[6:134] + w[1]*win[7:135] + w[0]*kfs[j]
            return ks * v_s[c, 128*j:128*(j+1), :].astype(f32)
        ties = []
        for jp in range(8):
            p = _pk(kvt(2*jp), kvt(2*jp+1)).reshape(16, 8, 128)
            kv_s[:, jp] = p
            ties += [pltpu.bitcast(p[i] & z_s[...], f32) for i in range(16)]
        return ties

    def PF(c):
        for jp in range(8):
            ha = hf_s[c, :, 256*jp:256*jp+128].astype(f32)
            hb = hf_s[c, :, 256*jp+128:256*jp+256].astype(f32)
            ht_s[:, jp] = _pk(ha, hb).T.reshape(16, 8, 128)

    def tied(p, ties, lo, hi, idx):
        mine = [t for qi, t in enumerate(ties) if lo + (qi*(hi-lo))//len(ties) == idx]
        if not mine:
            return p
        rows = [p[8*i:8*i+8] for i in range(p.shape[0]//8)]
        for i, t in enumerate(mine):
            if p.dtype == u32:
                rows[i % len(rows)] = rows[i % len(rows)] | t
            else:
                rows[-1-i] = rows[-1-i] + pltpu.bitcast(t, f32)
        return jnp.concatenate(rows, axis=0)

    def FT(c, slot=0):
        for j in range(16):
            t = hf_s[c, :, 128*j:128*(j+1)].astype(f32).T
            if j == 0 and E("DF"):
                cs = pl.ds(_mo(c*128, 128), 128)
                first = jax.lax.broadcasted_iota(i32, (8, 128), 0) == 0
                t = jnp.concatenate([t[0:8] + jnp.where(first, skf_s[4:5, cs], 0.0), t[8:]], axis=0)
            hT_s[slot, j] = t

    def FV(slot=0):
        ties = []
        for g in range(8):
            for b in range(2):
                a = [hT_s[slot, n1//2, 64*(n1 % 2) + 8*g:64*(n1 % 2) + 8*g + 8, :] for n1 in range(32)]
                CH = int(E("CH", "0"))
                if CH and len(ties) >= CH:
                    tz = pltpu.bitcast(ties[-CH], f32)
                    a = [x + tz if True else x for i, x in enumerate(a)]
                X = branch(a, b)
                ps = []
                for m in range(16):
                    kap = 2*m + b
                    p = _pk(X[m][0], X[m][1])
                    s2_s[1, kap // 16, kap % 16, g] = p
                    ps.append(p)
                while len(ps) > 1:
                    ps = [ps[i] | ps[i+1] for i in range(0, len(ps), 2)]
                ties.append(ps[0] & z_s[...])
        return ties

    F0 = int(E("F0", "4")); F1 = int(E("F1", "40"))
    def S1(srcs=(0, 1), ties=()):
        for src in srcs:
            buf = (kv_s, ht_s)[src]
            for g in range(8):
                lo = _dot(_tob(G_s[0]), _tob(tied(buf[g].reshape(64, 128), ties, F0, F1, 2*g)))
                hi = _dot(_tob(G_s[1]), _tob(tied(buf[8+g].reshape(64, 128), ties, F0, F1, 2*g+1)))
                for par, e in enumerate((lo+hi, lo-hi)):
                    e = e.reshape(16, 2, 8, 128)
                    s2_s[src, par, :, g] = _pk(e[:, 0], e[:, 1])

    def S2(c, ties):
        cs = pl.ds(_mo(c*128, 128), 128)
        dd = skf_s[4:5, cs]
        NP = 32 - TIE0
        def AB(k1):
            Ys = []
            for par in range(2):
                Hm = _tob(H_s[2*k1+par])
                A = _dot(Hm, _tob(s2_s[0, par, k1].reshape(64, 128)))
                B = _dot(Hm, _tob(s2_s[1, par, k1].reshape(64, 128)))
                Ar, Ai, Br, Bi = A[:64], A[64:], B[:64] if E('DF') else B[:64] + dd, B[64:]
                Yr = Ar*Br - Ai*Bi
                Yi = Ar*Bi + Ai*Br
                if ties:
                    n = 2*k1 + par
                    mine = [t for qi, t in enumerate(ties) if (qi*NP)//len(ties) + TIE0 == n]
                    rows = [Yr[8*i:8*i+8] for i in range(8)]
                    for i, t in enumerate(mine):
                        rows[i % 8] = rows[i % 8] + t
                    Yr = jnp.concatenate(rows, axis=0)
                Ys.append(jnp.concatenate([Yr, Yi], axis=0).astype(bf16))
            return Ys
        def DD(k1, Ys):
            Dd = [_dot(_tob(HI_s[2*k1+par]), Ys[par]) for par in range(2)]
            for lh, e in enumerate((Dd[0] + Dd[1], Dd[0] - Dd[1])):
                s3_s[lh, :, k1] = _pk(e[0:64], e[64:128]).reshape(8, 8, 128)
        pend = {}
        for k1 in range(16 + LAG):
            if k1 < 16:
                pend[k1] = AB(k1)
            if k1 - LAG >= 0:
                DD(k1 - LAG, pend.pop(k1 - LAG))

    def S3(c, ties=()):
        cs = pl.ds(_mo(c*128, 128), 128)
        for lh in range(2):
            for g in range(8):
                w = s3_s[lh, g].reshape(128, 128)
                w = jnp.concatenate([tied(w[0:64], ties, F0, F1, 16+4*(8*lh+g)//2), tied(w[64:128], ties, F0, F1, 17+4*(8*lh+g)//2)], axis=0) if ties else w
                o = _dot(_tob(GI_s[lh]), _tob(w))
                l0 = 64*lh + 8*g
                for j in range(16):
                    y_s[128*j+l0:128*j+l0+8, cs] = o[8*j:8*j+8]

    with scope("s1_waith"):
        cp_h(0).wait(); cp_sk.wait(); cp_d.wait()
        skf_s[0:4, :] = sk_s[...].astype(f32)
        skf_s[4:5, :] = d_s[...].astype(f32).reshape(1, D)
    with scope("s2_prof"):
        if E('FV'):
            FT(0); FV()
        else:
            PF(0); S1((1,))
    with scope("s3_waitkv"):
        cp_k(0).wait(); cp_v(0).wait()
    with scope("s3b_prokv"):
        P(0); S1((0,))
        if E('FT2'):
            cp_h(1).wait()
            FT(1, 1)
    def conv_body(c, carry):
        cp_k(c+1).wait(); cp_v(c+1).wait()
        if E("FT2"):
            @pl.when(c < 3)
            def _():
                cp_h(c+2).wait()
        elif not E("HW2"):
            cp_h(c+1).wait()
        if E('FV'):
            ties = P(c+1)
            if E("FT1"): FT(c+1)
            S2(c, ties)
            def second():
                if E("HW2"): cp_h(c+1).wait()
                if E("FT2"):
                    tf = FV((c+1) % 2)
                    FT(jnp.minimum(c+2, 4), c % 2)
                else:
                    if not E("FT1"): FT(c+1)
                    tf = FV()
                if not E("NOT"):
                    S1((0,), tf); S3(c, tf)
                else:
                    S1((0,)); S3(c)
            if E("BAR"):
                pl.when(flag_s[0] == 1)(second)
            else:
                second()
        else:
            ties = P(c+1); PF(c+1); S2(c, ties); S1(); S3(c)
        return carry
    with scope("s4_convloop"):
        jax.lax.fori_loop(0, 4, conv_body, 0)
    with scope("s5_wait"):
        cp_q[0].wait()
        for cp in cp_w[0]: cp.wait()

    lane = jax.lax.broadcasted_iota(i32, (TM, 128), 1)

    def or_ties(val):
        ab = pltpu.bitcast(val, u32)
        out = []
        for g in range(0, val.shape[0], 8):
            t = ab[g:g+8, 0:128]
            for k in range(1, 5):
                t = t | ab[g:g+8, 128*k:128*(k+1)]
            out.append(t & z_s[...])
        return out

    def A0(r0, nrows):
        lnx, ties = {}, []
        for j in range(0, nrows, ACH):
            n = min(ACH, nrows - j)
            lnx[r0 + j] = _ln(q_s[pl.ds(r0 + j, n), :].astype(f32))
            ties += [pltpu.bitcast(t, f32) for t in or_ties(lnx[r0 + j])]
        return lnx, ties

    def A(r0, nrows, lnx=None):
        ties = []
        for j in range(0, nrows, ACH):
            n = min(ACH, nrows - j)
            r = pl.ds(_mo(r0 + j, 16), n)
            x = q_s[r, :].astype(f32)
            h = x + (lnx[r0 + j] if lnx else _ln(x))*y_s[r, :]
            h_s[r, :] = h
            if E("CF"):
                m = jnp.sum(h, axis=-1, keepdims=True) * (1.0/D)
                c = h - m
                var = jnp.sum(c*c, axis=-1, keepdims=True) * (1.0/D)
                rs = jax.lax.rsqrt(var + 1e-5)
                xp = c * rs
                a = xp * jax.lax.rsqrt(var*rs*rs + 1e-5)
            else:
                xp = _ln(h)
                a = _ln(xp)
            xp_s[r, :] = xp
            a_s[r, :] = a
            ties += or_ties(a)
        return ties

    def M1(r0, nrows, ties=()):
        r = pl.ds(r0, nrows)
        av = [a_s[r, k*128:(k+1)*128].astype(bf16) for k in range(5)]
        for n in range(5):
            acc = None
            for k in range(5):
                w = tied(w1_s[n, k*64:(k+1)*64, :], ties, int(E("U0", "3")), int(E("U1", "25")), n*5+k)
                p = _dot(av[k], _tob(w))
                acc = p if acc is None else acc + p
            hh_s[n, pl.ds(r0+8, nrows), :] = _gelu(acc)

    def M2(base):
        r = pl.ds(base, TM)
        def sh(n, s): return hh_s.at[n, pl.ds(base, TM+16), :][8-s:8-s+TM, :]
        gs = [sh(0, 1),
              jnp.where(lane < 32, sh(1, 1), sh(1, -1)),
              jnp.where(lane < 64, sh(2, -1), sh(2, 2)),
              jnp.where(lane < 96, sh(3, 2), sh(3, -2)),
              sh(4, -2)]
        gs = [g.astype(bf16) for g in gs]
        x1s = []
        for n in range(5):
            acc = None
            for k in range(5):
                p = _dot(gs[k], _tob(w2_s[n, k*64:(k+1)*64, :]))
                acc = p if acc is None else acc + p
            x1s.append(xp_s[r, n*128:(n+1)*128] + acc)
        x1 = jnp.concatenate(x1s, axis=1)
        res_s[...] = h_s[r, :] + x1
        return _ln(x1)

    def M3(b):
        bs = [b[:, k*128:(k+1)*128].astype(bf16) for k in range(5)]
        gs = []
        for n in range(14):
            lo, hi = n*64, min((n+1)*64, F//2)
            acc = None
            for k in range(5):
                p = _dot_t(bs[k], _tob(w3_s[k, lo:hi, :]))
                acc = p if acc is None else acc + p
            gs.append(_gelu(acc).astype(bf16))
        return gs

    def M4(slot, gs, ties=(), post=None):
        for n in range(5):
            acc = None
            for k in range(14):
                lo, hi = k*64, min((k+1)*64, F//2)
                if E("WT"):
                    p = _dot(gs[k], _tob(tied(w4_s[n, lo:hi, :], ties, T0, T1, n*14+k)))
                else:
                    p = _dot(gs[k], _tob(w4_s[n, lo:hi, :]))
                    p = tied(p, ties, T0, T1, n*14+k)
                acc = p if acc is None else acc + p
            cs = slice(n*128, (n+1)*128)
            o_s[slot, :, cs] = (res_s[:, cs] + acc).astype(bf16)
            if post: post(n)

    with scope("s6_convepi_mlppro"):
        if E("PRE"):
            lnx, ties0 = A0(0, TM+SK)
            l2, t2 = A0(TM+SK, TM)
            lnx.update(l2); ties0 += t2
            S2(4, ties0); S3(4)
        else:
            lnx = None
            S2(4, None); S3(4)
        A(0, TM+SK, lnx)
        ties = A(TM+SK, TM, lnx)
        M1(0, TM+SK, ties if E("U0") else ())
    with scope("s8_waitw"):
        for wi in (1, 2, 3):
            for cp in cp_w[wi]: cp.wait()
        cp_q[1].wait()

    def mlp_body(i, carry):
        slot = i % 2
        @pl.when(i >= 2)
        def _():
            cp_o(i-2, slot).wait()
        base = _mo(i*TM, TM)
        a1 = _mo((i+1)*TM+SK, SK)
        a2 = _mo(jnp.minimum(i+2, NT-1)*TM+SK, SK)
        b = M2(base); M1(a1, TM); gs = M3(b); ties = A(a2, TM); M4(slot, gs, ties)
        cp_o(i, slot).start()
        return carry
    with scope("s9_mlploop"):
        jax.lax.fori_loop(0, NT-1, mlp_body, 0)
    i = NT-1
    with scope("sA_mlpepi"):
        cp_o(i-2, i % 2).wait()
        b = M2(i*TM)
        if E("SLAB"):
            M4(i % 2, M3(b), post=lambda n: cp_slab(i, n).start())
        else:
            M4(i % 2, M3(b))
            cp_o(i, i % 2).start()
    with scope("sB_final"):
        cp_o(i-1, (i-1) % 2).wait()
        if E("SLAB"):
            for n in range(5): cp_slab(i, n).wait()
        else:
            cp_o(i, i % 2).wait()


def _hbm(x):
    return pltpu.with_memory_space_constraint(x, pltpu.HBM)


@jax.jit
def pallas_sequential_preLN__ssm_conv_h3__mixer_s_mlp__prompt_kernel(
    A_q, A_k, A_v, A_shift_k, A_ssm_k, A_ssm_D, B_x, B_w1, B_w2, B_w3, B_w4):
    del B_x
    args = (A_q.reshape(S, D), A_k.reshape(S, D), A_v.reshape(S, D), A_shift_k.T, A_ssm_k, A_ssm_D,
            B_w1, B_w2, B_w3.T, B_w4)
    out = pl.pallas_call(
        _kernel,
        out_shape=jax.ShapeDtypeStruct((S, D), bf16),
        in_specs=[pl.BlockSpec(memory_space=pltpu.HBM)] * len(args),
        out_specs=pl.BlockSpec(memory_space=pltpu.HBM),
        scratch_shapes=[
            pltpu.VMEM((5, S, 128), bf16), pltpu.VMEM((5, S, 128), bf16), pltpu.VMEM((5, 128, S), bf16),
            pltpu.VMEM((4, D), bf16), pltpu.VMEM((D,), bf16), pltpu.VMEM((8, D), f32),
            pltpu.VMEM((2, 128, 128), u32), pltpu.VMEM((32, 64, 128), u32), pltpu.VMEM((32, 64, 128), u32), pltpu.VMEM((2, 64, 256), u32),
            pltpu.VMEM((16, 8, 8, 128), u32), pltpu.VMEM((16, 8, 8, 128), u32),
            pltpu.VMEM((2, 2, 16, 8, 8, 128), u32), pltpu.VMEM((2, 8, 16, 8, 128), u32),
            pltpu.VMEM((8, 128), u32), pltpu.VMEM((S+SK, D), f32),
            pltpu.VMEM((S+8, 128), f32), pltpu.VMEM((2, 16, 128, 128), f32), pltpu.VMEM((S+SK, D), bf16),
            pltpu.VMEM((5, D//2, 128), u32), pltpu.VMEM((5, D//2, 128), u32), pltpu.VMEM((5, F//2, 128), u32), pltpu.VMEM((5, F//2, 128), u32),
            pltpu.VMEM((S+SK, D), f32), pltpu.VMEM((S+SK, D), f32), pltpu.VMEM((S+SK, D), f32),
            pltpu.VMEM((5, S+SK+16, 128), f32), pltpu.VMEM((TM, D), f32), pltpu.VMEM((2, TM, D), bf16),
            pltpu.SMEM((4,), i32),
            pltpu.SemaphoreType.DMA((39,)), pltpu.SemaphoreType.DMA((7,)),
        ],
        compiler_params=pltpu.CompilerParams(vmem_limit_bytes=100*2**20),
        name="ssm_mixer_block",
    )(*[_hbm(a) for a in args])
    return out.reshape(1, S, D)
```

```python
import numpy as np
import jax
import jax.numpy as jnp
import jax.experimental.pallas as pl
import jax.experimental.pallas.tpu as pltpu

S, D, F = 2048, 640, 1728
TM = 256
NT = S // TM
SK = 16
ACH = 32
LAG = 3
TIE0 = 1
T0, T1 = 6, 62
F0, F1 = 14, 48
NH = 2
f32, bf16, u32, i32 = jnp.float32, jnp.bfloat16, jnp.uint32, jnp.int32


def _cmul(a, b):
    return a[0]*b[0] - a[1]*b[1], a[0]*b[1] + a[1]*b[0]


def _cis(m):
    mm = (m & 8191) + 1024
    q = mm >> 11
    x = ((mm & 2047) - 1024).astype(f32) * np.float32(2*np.pi/8192)
    x2 = x*x
    s = x + x*x2*(np.float32(-1/6) + x2*(np.float32(1/120) + x2*(np.float32(-1/5040) + x2*np.float32(1/362880))))
    c = 1.0 + x2*(np.float32(-1/2) + x2*(np.float32(1/24) + x2*(np.float32(-1/720) + x2*(np.float32(1/40320) + x2*np.float32(-1/3628800)))))
    odd = (q & 1) == 1
    cs = jnp.where(odd, s, c); sn = jnp.where(odd, c, s)
    cs = jnp.where(((q + 1) & 2) != 0, -cs, cs)
    sn = jnp.where((q & 2) != 0, -sn, sn)
    return cs, sn


def sadd(a, b):
    (sa, xa), (sb, xb) = a, b
    if sa == sb: return (sa, xa + xb)
    return (1, xa - xb) if sa > 0 else (1, xb - xa)
def sneg(a): return (-a[0], a[1])
def ssub(a, b): return sadd(a, sneg(b))
def smul(a, c):
    c = float(c)
    return (a[0]*(1 if c > 0 else -1), a[1]*np.float32(abs(c)))
def val(a):
    if a[0] > 0: return a[1]
    return -a[1]
def cadd(a, b): return (sadd(a[0], b[0]), sadd(a[1], b[1]))
def csub(a, b): return (ssub(a[0], b[0]), ssub(a[1], b[1]))
def cmuli(a): return (sneg(a[1]), a[0])
def bfly4(z0, z1, z2, z3):
    t0, t1, t2, t3 = cadd(z0, z2), csub(z0, z2), cadd(z1, z3), csub(z1, z3)
    it3 = cmuli(t3)
    return cadd(t0, t2), cadd(t1, it3), csub(t0, t2), csub(t1, it3)
def ctw(a, k):
    k %= 16
    if k == 0: return a
    if k == 4: return cmuli(a)
    if k == 8: return (sneg(a[0]), sneg(a[1]))
    if k == 12: return (a[1], sneg(a[0]))
    c, s = np.cos(2*np.pi*k/16), np.sin(2*np.pi*k/16)
    if k % 2 == 0:
        r = sadd((a[0][0]*int(np.sign(c)), a[0][1]), (-a[1][0]*int(np.sign(s)), a[1][1]))
        i = sadd((a[0][0]*int(np.sign(s)), a[0][1]), (a[1][0]*int(np.sign(c)), a[1][1]))
        return (smul(r, abs(c)), smul(i, abs(c)))
    return (ssub(smul(a[0], c), smul(a[1], s)), sadd(smul(a[0], s), smul(a[1], c)))
def fft16(z):
    u = [bfly4(z[n1], z[4+n1], z[8+n1], z[12+n1]) for n1 in range(4)]
    X = [None]*16
    for m1 in range(4):
        v = [ctw(u[n1][m1], m1*n1) for n1 in range(4)]
        o = bfly4(*v)
        for m2 in range(4): X[m1 + 4*m2] = o[m2]
    return X
def branch(a, b):
    e1, e2 = (1, 16) if b == 0 else (5, 80)
    z = []
    for n in range(16):
        a0, a1 = (1, a[n]), (1, a[n+16])
        if n == 0:
            c = np.cos(2*np.pi*e2/128); s = np.sin(2*np.pi*e2/128)
            t = smul(a1, abs(c))
            z.append((sadd(a0, (t[0]*int(np.sign(c)), t[1])), (t[0]*int(np.sign(s)), t[1])))
        else:
            al, be = 2*np.pi*(e1*n)/128, 2*np.pi*(e1*n + e2)/128
            z.append((sadd(smul(a0, np.cos(al)), smul(a1, np.cos(be))), sadd(smul(a0, np.sin(al)), smul(a1, np.sin(be)))))
    X = fft16(z)
    return [(val(x[0]), val(x[1])) for x in X]


def _dot(a, b):
    return jnp.dot(a, b, preferred_element_type=f32)

def _dot_t(a, b):
    return jax.lax.dot_general(a, b, (((1,), (1,)), ((), ())), preferred_element_type=f32)

def _tob(w):
    return pltpu.bitcast(w, bf16)

def _pk(a, b):
    return pltpu.pack_elementwise([a, b], packed_dtype=bf16)

def _mo(v, m):
    return v if isinstance(v, int) else pl.multiple_of(v, m)

def _ln(x):
    m = jnp.sum(x, axis=-1, keepdims=True) * (1.0/D)
    c = x - m
    v = jnp.sum(c*c, axis=-1, keepdims=True) * (1.0/D)
    return c * jax.lax.rsqrt(v + 1e-5)

def _gelu(x):
    return (0.5*x)*(1.0 + jnp.tanh(x*(0.7978845608028654 + (0.7978845608028654*0.044715)*(x*x))))


def _kernel(q_hbm, k_hbm, v_hbm, sk_hbm, h_hbm, d_hbm, w1_hbm, w2_hbm, w3_hbm, w4_hbm, o_hbm,
            k_s, v_s, hf_s, sk_s, d_s, skf_s, G_s, H_s, HI_s, GI_s, kv_s, s2_s, s3_s, z_s, y_s,
            hT_s, q_s, w1_s, w2_s, w3_s, w4_s, h_s, xp_s, a_s, hh_s, res_s, o_s,
            flag_s, sem, sem_o):
    def cp_k(c): return pltpu.make_async_copy(k_hbm.at[:, pl.ds(_mo(c*128, 128), 128)], k_s.at[c], sem.at[c])
    def cp_v(c): return pltpu.make_async_copy(v_hbm.at[:, pl.ds(_mo(c*128, 128), 128)], v_s.at[c], sem.at[5+c])
    def cp_h(c): return pltpu.make_async_copy(h_hbm.at[pl.ds(_mo(c*128, 128), 128), :], hf_s.at[c], sem.at[10+c])
    HR = S // NH
    cp_kv0 = [pltpu.make_async_copy(hbm.at[pl.ds(i*HR, HR), pl.ds(0, 128)], buf.at[0, pl.ds(i*HR, HR)], sem.at[39 + 2*i + w])
              for i in range(NH) for w, (hbm, buf) in enumerate(((k_hbm, k_s), (v_hbm, v_s)))]
    cp_sk = pltpu.make_async_copy(sk_hbm, sk_s, sem.at[15])
    cp_d = pltpu.make_async_copy(d_hbm, d_s, sem.at[16])
    QB = (0, 640, S)
    cp_q = [pltpu.make_async_copy(q_hbm.at[pl.ds(QB[i], QB[i+1]-QB[i]), :], q_s.at[pl.ds(QB[i], QB[i+1]-QB[i]), :], sem.at[17+i])
            for i in range(2)]
    cp_w = []
    for wi, (w_hbm, w_s) in enumerate(((w1_hbm, w1_s), (w2_hbm, w2_s), (w3_hbm, w3_s), (w4_hbm, w4_s))):
        wv = w_s.bitcast(bf16)
        cp_w.append([pltpu.make_async_copy(w_hbm.at[:, pl.ds(128*n, 128)], wv.at[n], sem.at[19+5*wi+n]) for n in range(5)])
    def cp_o(i, slot):
        return pltpu.make_async_copy(o_s.at[slot], o_hbm.at[pl.ds(_mo(i*TM, TM), TM), :], sem_o.at[slot])
    def cp_slab(i, n):
        return pltpu.make_async_copy(o_s.at[i % 2, :, pl.ds(128*n, 128)], o_hbm.at[pl.ds(i*TM, TM), pl.ds(128*n, 128)], sem_o.at[2+n])

    for cp in (cp_h(0), cp_sk, cp_d, *cp_kv0, cp_k(1), cp_v(1), cp_h(1)):
        cp.start()
    for c in range(2, 5):
        cp_k(c).start(); cp_v(c).start(); cp_h(c).start()
    cp_q[0].start()
    for wi in range(4):
        for cp in cp_w[wi]:
            cp.start()
    cp_q[1].start()

    def gen_G():
        lane = jax.lax.broadcasted_iota(i32, (8, 128), 1)
        row = jax.lax.broadcasted_iota(i32, (8, 128), 0)
        ri = row >> 2; rr = row & 3
        j = 2*(lane >> 4) + (lane & 1); rp = (lane >> 1) & 7
        for lh in range(2):
            n1 = 2*j + lh
            W = _cis(n1*64 - 2048*ri); u = _cis(n1*256)
            for k1 in range(16):
                G_s[lh, 8*k1:8*k1+8, :] = _pk(jnp.where(2*rr == rp, W[0], 0.0), jnp.where(2*rr + 1 == rp, W[0], 0.0))
                if k1 < 15: W = _cmul(W, u)
    def gen_GI():
        lane = jax.lax.broadcasted_iota(i32, (8, 256), 1)
        row = jax.lax.broadcasted_iota(i32, (8, 256), 0)
        jo = row >> 2; rr = row & 3
        k1 = lane >> 4; r = (lane >> 1) & 7; ri = lane & 1
        u = _cis((4*k1 + 1)*256)
        for lh in range(2):
            W = _cis((4*k1 + 1)*(2*jo + lh)*64 - 2048*ri)
            for jp in range(8):
                v = W[0] * (1.0/S)
                GI_s[lh, 8*jp:8*jp+8, :] = _pk(jnp.where(2*rr == r, v, 0.0), jnp.where(2*rr + 1 == r, v, 0.0))
                if jp < 7: W = _cmul(W, u)
    def gen_H():
        lane = jax.lax.broadcasted_iota(i32, (32, 128), 1)
        row = jax.lax.broadcasted_iota(i32, (32, 128), 0)
        l = lane >> 1; ri = lane & 1
        u = _cis(4*l[0:8]); u = tuple(jnp.concatenate([x]*4, axis=0) for x in u)
        W = [_cis((1 + 256*row + 128*p)*l + 2048*ri) for p in range(2)]
        for n in range(32):
            idx = 2*(n % 16) + n // 16
            H_s[idx, 0:32, :] = _pk(W[0][0], W[1][0])
            H_s[idx, 32:64, :] = _pk(W[0][1], W[1][1])
            if n < 31: W = [_cmul(w, u) for w in W]
        k2 = lane & 63; rip = lane >> 6
        T = [_cis(-4*(2*row + p)) for p in range(2)]
        W = [_cis(-(1 + 128*k2)*(2*row + p) + 2048*rip) for p in range(2)]
        for n in range(32):
            idx = 2*(n % 16) + n // 16
            HI_s[idx, 0:32, :] = _pk(W[0][0], W[1][0])
            HI_s[idx, 32:64, :] = _pk(W[0][1], W[1][1])
            if n < 31: W = [_cmul(w, t) for w, t in zip(W, T)]
    gen_G(); gen_H(); gen_GI()
    flag_s[0] = 1
    z_s[...] = jnp.zeros((8, 128), u32)
    hh_s[:, 0:8, :] = jnp.zeros((5, 8, 128), f32)
    q_s[S:S+SK, :] = jnp.zeros((SK, D), bf16)
    y_s[S:S+SK, :] = jnp.zeros((SK, D), f32)

    def P(c, jps=range(8)):
        cs = pl.ds(_mo(c*128, 128), 128)
        w = [skf_s[i:i+1, cs] for i in range(4)]
        kfs = {j: k_s[c, 128*j:128*(j+1), :].astype(f32) for j in range(max(2*jps[0]-1, 0), 2*jps[-1]+2)}
        def kvt(j):
            prev = kfs[j-1][120:128] if j else jnp.zeros((8, 128), f32)
            win = jnp.concatenate([prev, kfs[j]], axis=0)
            ks = w[3]*win[5:133] + w[2]*win[6:134] + w[1]*win[7:135] + w[0]*kfs[j]
            return ks * v_s[c, 128*j:128*(j+1), :].astype(f32)
        ties = []
        for jp in jps:
            p = _pk(kvt(2*jp), kvt(2*jp+1)).reshape(16, 8, 128)
            kv_s[:, jp] = p
            ties += [pltpu.bitcast(p[i] & z_s[...], f32) for i in range(16)]
        return ties

    def tied(p, ties, lo, hi, idx):
        mine = [t for qi, t in enumerate(ties) if lo + (qi*(hi-lo))//len(ties) == idx]
        if not mine:
            return p
        rows = [p[8*i:8*i+8] for i in range(p.shape[0]//8)]
        for i, t in enumerate(mine):
            rows[i % len(rows)] = rows[i % len(rows)] | t
        return jnp.concatenate(rows, axis=0)

    def FT(c):
        for j in range(16):
            t = hf_s[c, :, 128*j:128*(j+1)].astype(f32).T
            if j == 0:
                cs = pl.ds(_mo(c*128, 128), 128)
                first = jax.lax.broadcasted_iota(i32, (8, 128), 0) == 0
                t = jnp.concatenate([t[0:8] + jnp.where(first, skf_s[4:5, cs], 0.0), t[8:]], axis=0)
            hT_s[j] = t

    def FV():
        ties = []
        for g in range(8):
            for b in range(2):
                a = [hT_s[n1//2, 64*(n1 % 2) + 8*g:64*(n1 % 2) + 8*g + 8, :] for n1 in range(32)]
                X = branch(a, b)
                ps = []
                for m in range(16):
                    kap = 2*m + b
                    p = _pk(X[m][0], X[m][1])
                    s2_s[1, kap // 16, kap % 16, g] = p
                    ps.append(p)
                while len(ps) > 1:
                    ps = [ps[i] | ps[i+1] for i in range(0, len(ps), 2)]
                ties.append(ps[0] & z_s[...])
        return ties

    def S1(ties=()):
        for g in range(8):
            lo = _dot(_tob(G_s[0]), _tob(tied(kv_s[g].reshape(64, 128), ties, F0, F1, 2*g)))
            hi = _dot(_tob(G_s[1]), _tob(tied(kv_s[8+g].reshape(64, 128), ties, F0, F1, 2*g+1)))
            for par, e in enumerate((lo+hi, lo-hi)):
                e = e.reshape(16, 2, 8, 128)
                s2_s[0, par, :, g] = _pk(e[:, 0], e[:, 1])

    def S2(c, ties):
        NP = 32 - TIE0
        def AB(k1):
            Ys = []
            for par in range(2):
                Hm = _tob(H_s[2*k1+par])
                A = _dot(Hm, _tob(s2_s[0, par, k1].reshape(64, 128)))
                B = _dot(Hm, _tob(s2_s[1, par, k1].reshape(64, 128)))
                Ar, Ai, Br, Bi = A[:64], A[64:], B[:64], B[64:]
                Yr = Ar*Br - Ai*Bi
                Yi = Ar*Bi + Ai*Br
                if ties:
                    n = 2*k1 + par
                    mine = [t for qi, t in enumerate(ties) if (qi*NP)//len(ties) + TIE0 == n]
                    rows = [Yr[8*i:8*i+8] for i in range(8)]
                    for i, t in enumerate(mine):
                        rows[i % 8] = rows[i % 8] + t
                    Yr = jnp.concatenate(rows, axis=0)
                Ys.append(jnp.concatenate([Yr, Yi], axis=0).astype(bf16))
            return Ys
        def DD(k1, Ys):
            Dd = [_dot(_tob(HI_s[2*k1+par]), Ys[par]) for par in range(2)]
            for lh, e in enumerate((Dd[0] + Dd[1], Dd[0] - Dd[1])):
                s3_s[lh, :, k1] = _pk(e[0:64], e[64:128]).reshape(8, 8, 128)
        pend = {}
        for k1 in range(16 + LAG):
            if k1 < 16:
                pend[k1] = AB(k1)
            if k1 - LAG >= 0:
                DD(k1 - LAG, pend.pop(k1 - LAG))

    def S3(c, ties=()):
        cs = pl.ds(_mo(c*128, 128), 128)
        for lh in range(2):
            for g in range(8):
                w = s3_s[lh, g].reshape(128, 128)
                w = jnp.concatenate([tied(w[0:64], ties, F0, F1, 16+4*(8*lh+g)//2), tied(w[64:128], ties, F0, F1, 17+4*(8*lh+g)//2)], axis=0) if ties else w
                o = _dot(_tob(GI_s[lh]), _tob(w))
                l0 = 64*lh + 8*g
                for j in range(16):
                    y_s[128*j+l0:128*j+l0+8, cs] = o[8*j:8*j+8]

    cp_h(0).wait(); cp_sk.wait(); cp_d.wait()
    skf_s[0:4, :] = sk_s[...].astype(f32)
    skf_s[4:5, :] = d_s[...].astype(f32).reshape(1, D)
    FT(0); FV()
    for i in range(NH):
        cp_kv0[2*i].wait(); cp_kv0[2*i+1].wait()
        P(0, range(i*8//NH, (i+1)*8//NH))
    S1()

    def conv_body(c, carry):
        cp_k(c+1).wait(); cp_v(c+1).wait()
        ties = P(c+1)
        S2(c, ties)
        @pl.when(flag_s[0] == 1)
        def _():
            cp_h(c+1).wait()
            FT(c+1)
            tf = FV()
            S1(tf); S3(c, tf)
        return carry
    jax.lax.fori_loop(0, 4, conv_body, 0)
    cp_q[0].wait()
    for cp in cp_w[0]: cp.wait()

    lane = jax.lax.broadcasted_iota(i32, (TM, 128), 1)

    def or_ties(val):
        ab = pltpu.bitcast(val, u32)
        out = []
        for g in range(0, val.shape[0], 8):
            t = ab[g:g+8, 0:128]
            for k in range(1, 5):
                t = t | ab[g:g+8, 128*k:128*(k+1)]
            out.append(t & z_s[...])
        return out

    def A0(r0, nrows):
        lnx, ties = {}, []
        for j in range(0, nrows, ACH):
            n = min(ACH, nrows - j)
            lnx[r0 + j] = _ln(q_s[pl.ds(r0 + j, n), :].astype(f32))
            ties += [pltpu.bitcast(t, f32) for t in or_ties(lnx[r0 + j])]
        return lnx, ties

    def A(r0, nrows, lnx=None):
        ties = []
        for j in range(0, nrows, ACH):
            n = min(ACH, nrows - j)
            r = pl.ds(_mo(r0 + j, 16), n)
            x = q_s[r, :].astype(f32)
            h = x + (lnx[r0 + j] if lnx else _ln(x))*y_s[r, :]
            h_s[r, :] = h
            xp = _ln(h)
            a = _ln(xp)
            xp_s[r, :] = xp
            a_s[r, :] = a
            ties += or_ties(a)
        return ties

    def M1(r0, nrows):
        r = pl.ds(r0, nrows)
        av = [a_s[r, k*128:(k+1)*128].astype(bf16) for k in range(5)]
        for n in range(5):
            acc = None
            for k in range(5):
                p = _dot(av[k], _tob(w1_s[n, k*64:(k+1)*64, :]))
                acc = p if acc is None else acc + p
            hh_s[n, pl.ds(r0+8, nrows), :] = _gelu(acc)

    def M2(base):
        r = pl.ds(base, TM)
        def sh(n, s): return hh_s.at[n, pl.ds(base, TM+16), :][8-s:8-s+TM, :]
        gs = [sh(0, 1),
              jnp.where(lane < 32, sh(1, 1), sh(1, -1)),
              jnp.where(lane < 64, sh(2, -1), sh(2, 2)),
              jnp.where(lane < 96, sh(3, 2), sh(3, -2)),
              sh(4, -2)]
        gs = [g.astype(bf16) for g in gs]
        x1s = []
        for n in range(5):
            acc = None
            for k in range(5):
                p = _dot(gs[k], _tob(w2_s[n, k*64:(k+1)*64, :]))
                acc = p if acc is None else acc + p
            x1s.append(xp_s[r, n*128:(n+1)*128] + acc)
        x1 = jnp.concatenate(x1s, axis=1)
        res_s[...] = h_s[r, :] + x1
        return _ln(x1)

    def M3(b):
        bs = [b[:, k*128:(k+1)*128].astype(bf16) for k in range(5)]
        gs = []
        for n in range(14):
            lo, hi = n*64, min((n+1)*64, F//2)
            acc = None
            for k in range(5):
                p = _dot_t(bs[k], _tob(w3_s[k, lo:hi, :]))
                acc = p if acc is None else acc + p
            gs.append(_gelu(acc).astype(bf16))
        return gs

    def M4(slot, gs, ties=(), post=None):
        for n in range(5):
            acc = None
            for k in range(14):
                lo, hi = k*64, min((k+1)*64, F//2)
                p = _dot(gs[k], _tob(tied(w4_s[n, lo:hi, :], ties, T0, T1, n*14+k)))
                acc = p if acc is None else acc + p
            cs = slice(n*128, (n+1)*128)
            o_s[slot, :, cs] = (res_s[:, cs] + acc).astype(bf16)
            if post: post(n)

    lnx, ties0 = A0(0, TM+SK)
    l2, t2 = A0(TM+SK, TM)
    lnx.update(l2)
    S2(4, ties0 + t2); S3(4)
    A(0, TM+SK, lnx)
    A(TM+SK, TM, lnx)
    M1(0, TM+SK)
    for wi in (1, 2, 3):
        for cp in cp_w[wi]: cp.wait()
    cp_q[1].wait()

    def mlp_body(i, carry):
        slot = i % 2
        @pl.when(i >= 2)
        def _():
            cp_o(i-2, slot).wait()
        base = _mo(i*TM, TM)
        a1 = _mo((i+1)*TM+SK, SK)
        a2 = _mo(jnp.minimum(i+2, NT-1)*TM+SK, SK)
        b = M2(base); M1(a1, TM); gs = M3(b); ties = A(a2, TM); M4(slot, gs, ties)
        cp_o(i, slot).start()
        return carry
    jax.lax.fori_loop(0, NT-1, mlp_body, 0)
    i = NT-1
    cp_o(i-2, i % 2).wait()
    b = M2(i*TM)
    M4(i % 2, M3(b), post=lambda n: cp_slab(i, n).start())
    cp_o(i-1, (i-1) % 2).wait()
    for n in range(5):
        cp_slab(i, n).wait()


def _hbm(x):
    return pltpu.with_memory_space_constraint(x, pltpu.HBM)


@jax.jit
def pallas_sequential_preLN__ssm_conv_h3__mixer_s_mlp__prompt_kernel(
    A_q, A_k, A_v, A_shift_k, A_ssm_k, A_ssm_D, B_x, B_w1, B_w2, B_w3, B_w4):
    del B_x
    args = (A_q.reshape(S, D), A_k.reshape(S, D), A_v.reshape(S, D), A_shift_k.T, A_ssm_k, A_ssm_D,
            B_w1, B_w2, B_w3.T, B_w4)
    out = pl.pallas_call(
        _kernel,
        out_shape=jax.ShapeDtypeStruct((S, D), bf16),
        in_specs=[pl.BlockSpec(memory_space=pltpu.HBM)] * len(args),
        out_specs=pl.BlockSpec(memory_space=pltpu.HBM),
        scratch_shapes=[
            pltpu.VMEM((5, S, 128), bf16), pltpu.VMEM((5, S, 128), bf16), pltpu.VMEM((5, 128, S), bf16),
            pltpu.VMEM((4, D), bf16), pltpu.VMEM((D,), bf16), pltpu.VMEM((8, D), f32),
            pltpu.VMEM((2, 128, 128), u32), pltpu.VMEM((32, 64, 128), u32), pltpu.VMEM((32, 64, 128), u32), pltpu.VMEM((2, 64, 256), u32),
            pltpu.VMEM((16, 8, 8, 128), u32),
            pltpu.VMEM((2, 2, 16, 8, 8, 128), u32), pltpu.VMEM((2, 8, 16, 8, 128), u32),
            pltpu.VMEM((8, 128), u32), pltpu.VMEM((S+SK, D), f32),
            pltpu.VMEM((16, 128, 128), f32), pltpu.VMEM((S+SK, D), bf16),
            pltpu.VMEM((5, D//2, 128), u32), pltpu.VMEM((5, D//2, 128), u32), pltpu.VMEM((5, F//2, 128), u32), pltpu.VMEM((5, F//2, 128), u32),
            pltpu.VMEM((S+SK, D), f32), pltpu.VMEM((S+SK, D), f32), pltpu.VMEM((S+SK, D), f32),
            pltpu.VMEM((5, S+SK+16, 128), f32), pltpu.VMEM((TM, D), f32), pltpu.VMEM((2, TM, D), bf16),
            pltpu.SMEM((4,), i32),
            pltpu.SemaphoreType.DMA((39 + 2*NH,)), pltpu.SemaphoreType.DMA((7,)),
        ],
        compiler_params=pltpu.CompilerParams(vmem_limit_bytes=100*2**20),
        name="ssm_mixer_block",
    )(*[_hbm(a) for a in args])
    return out.reshape(1, S, D)
```
